```python
import jax
import jax.numpy as jnp

def _softmax(x, axis=-1):
    return jax.nn.softmax(x, axis=axis)
def _gelu(x):
    return jax.nn.gelu(x, approximate=True)
def _silu(x):
    return jax.nn.silu(x)
def _sigmoid(x):
    return jax.nn.sigmoid(x)
def _layernorm(x, axis=-1, eps=1e-5):
    m = jnp.mean(x, axis=axis, keepdims=True)
    v = jnp.var(x, axis=axis, keepdims=True)
    return (x - m) / jnp.sqrt(v + eps)
def _scatter_add(tgt, idx, src, axis=0):
    return tgt.at[idx].add(src)
def _segment_sum(src, seg, n):
    return jax.ops.segment_sum(src, seg, n)
class _Rng:
    def __init__(self, key):
        self._k = key
    def _next(self):
        self._k, sub = jax.random.split(self._k)
        return sub
    def normal(self, shape):
        return jax.random.normal(self._next(), shape, dtype=jnp.bfloat16)
    def randint(self, lo, hi, shape):
        return jax.random.randint(self._next(), shape, lo, hi, dtype=jnp.int32)
    def uniform(self, shape, lo=0.0, hi=1.0):
        return jax.random.uniform(self._next(), shape, jnp.bfloat16, lo, hi)
    def permutation(self, n):
        return jax.random.permutation(self._next(), n)


kernel_name = 'standalone__standard_2d_1d_3d_conv__vision'

def setup_inputs():
    _rng = _Rng(jax.random.key(int.from_bytes(__import__("os").urandom(4), "little")))
    _w = (lambda a: (lambda t: t.astype(jnp.bfloat16) if jnp.issubdtype(t.dtype, jnp.floating) else t)(jnp.asarray(a)))
    H = W = 384
    C = 384
    K = 1
    return {
        "x": _w((lambda *s: _rng.normal(s) * 0.05)(1, H, W, C)),
        "w": _w((lambda *s: _rng.normal(s) * 0.05)(K, K, C, C)),
        "b": _w((lambda *s: _rng.normal(s) * 0.05)(C)),
    }

def reference(x, w, b):
    B, H, W, Cin = x.shape
    K = w.shape[0]
    pl = (K - 1) // 2
    pr = K // 2
    xp = jnp.pad(x, ((0, 0), (pl, pr), (pl, pr), (0, 0)))
    out = sum(
        jnp.einsum('bhwc,cd->bhwd', xp[:, i:i+H, j:j+W, :], w[i, j])
        for i in range(K) for j in range(K)
    )
    return out + b[None, None, None, :]
```

```python
import jax
import jax.numpy as jnp
from jax import lax
import jax.experimental.pallas as pl
import jax.experimental.pallas.tpu as pltpu

_LANES = 128
_STREAM = 4096
_PAIR = 48

_READ_PIECE = 32
_READ_COPIES = ((5, 1), (1, 0)) * 2
_LAG = 12
_SWEEPS = 12
_PAIRS1 = 48
_LATE = 5

_WRITE_PIECE = 64
_WRITE_STREAMS = 6
_LEAD = 32
_WRITES = 19
_PAIRS2 = 96

_DOT_PAIRS = 12


def _matmul(view, w_ref, bias):
    m = view.shape[0] // _PAIR
    regs = pltpu.bitcast(view[...], jnp.uint32).reshape(m, 3, 8, _LANES)
    low = lax.broadcasted_iota(jnp.int32, (m, 8, _LANES), 1) < 4

    def dot(first, second, k):
        lhs = jnp.where(low, regs[:, first], regs[:, second]).reshape(8 * m, _LANES)
        acc = jnp.dot(
            pltpu.bitcast(lhs, view.dtype),
            w_ref[pl.ds(k * _LANES, _LANES), :],
            preferred_element_type=jnp.float32,
        )
        return acc.reshape(m, 2, 8, 3 * _LANES)

    y0, y1, y2 = dot(0, 1, 0), dot(2, 0, 1), dot(1, 2, 2)
    a = y0[:, 0] + y1[:, 1] + y2[:, 0] + bias
    b = y0[:, 1] + y1[:, 0] + y2[:, 1] + bias
    tiles = [t[:, :, n * _LANES:(n + 1) * _LANES] for t in (a, b) for n in range(3)]
    out = jnp.stack(tiles, axis=1).reshape(view.shape)
    view[...] = out.astype(view.dtype)


def _conv1x1_kernel(
    x_hbm, w_hbm, b_hbm, o_hbm, buf, w_ref, b_ref, group_sems, late_sem, out_sem
):
    n_streams = x_hbm.shape[0]
    streams = buf.reshape(x_hbm.shape)
    pairs = buf.shape[0] // _PAIR

    group = sum(n for n, _ in _READ_COPIES)
    groups = n_streams // group
    group_rows = group * _STREAM
    group_sweeps = _STREAM // _READ_PIECE
    sweeps = groups * group_sweeps
    head = _LAG + (sweeps - _LATE - _LAG) % _SWEEPS
    idle_steps = pl.cdiv(group_sweeps + _LAG - head, _SWEEPS) + 2
    first_sweep = head + idle_steps * _SWEEPS
    steps1 = (sweeps - _LATE - first_sweep) // _SWEEPS
    steps1 -= (pairs - steps1 * _PAIRS1) % _PAIRS2 // _PAIRS1
    steps2 = (pairs - steps1 * _PAIRS1) // _PAIRS2
    assert steps1 * _PAIRS1 + steps2 * _PAIRS2 == pairs

    group_writes = _STREAM // _WRITE_PIECE
    writes = n_streams // _WRITE_STREAMS * group_writes

    def wait(rows, sem):
        size = buf.at[pl.ds(0, rows)]
        pltpu.make_async_copy(size, size, sem).wait()

    def locate(i, per_group, piece):
        if isinstance(i, int):
            return i // per_group, i % per_group * piece
        shift = per_group.bit_length() - 1
        return i >> shift, pl.multiple_of((i & (per_group - 1)) * piece, piece)

    def read(sweep_of_thread, sem_of_thread=(None, None)):
        first = 0
        for n, thread in _READ_COPIES:
            if sweep_of_thread[thread] is not None:
                g, row = locate(sweep_of_thread[thread], group_sweeps, _READ_PIECE)
                idx = (pl.ds(g * group + first, n), pl.ds(row, _READ_PIECE))
                sem = sem_of_thread[thread]
                if sem is None:
                    sem = group_sems.at[g]
                copy = pltpu.make_async_copy(x_hbm.at[idx], streams.at[idx], sem)
                copy.start(priority=thread)
            first += n

    def write(i):
        g, row = locate(i, group_writes, _WRITE_PIECE)
        idx = (pl.ds(g * _WRITE_STREAMS, _WRITE_STREAMS), pl.ds(row, _WRITE_PIECE))
        copy = pltpu.make_async_copy(streams.at[idx], o_hbm.at[idx], out_sem)
        copy.start(priority=1)

    def compute(first_pair, n_pairs):
        row = pl.multiple_of(first_pair * _PAIR, 16)
        view = buf.at[pl.ds(row, n_pairs * _PAIR)]
        for i in range(0, n_pairs, _DOT_PAIRS):
            _matmul(view.at[pl.ds(i * _PAIR, _DOT_PAIRS * _PAIR)], w_ref, bias)

    w_copy = pltpu.make_async_copy(w_hbm, w_ref, out_sem)
    b_copy = pltpu.make_async_copy(b_hbm, b_ref, out_sem)
    read((None, 0))
    pl.loop(1, _LAG)(lambda i: read((None, i)))
    w_copy.start()
    b_copy.start()
    pl.loop(_LAG, first_sweep)(lambda i: read((i - _LAG, i)))
    w_copy.wait()
    b_copy.wait()
    bias = b_ref[...].astype(jnp.float32).reshape(1, -1)

    group_pairs = group_rows // _PAIR
    for i in range(steps1):
        g = ((i + 1) * _PAIRS1 - 1) // group_pairs
        assert (g + 1) * group_sweeps + _LAG <= first_sweep + (i + 1) * _SWEEPS
    groups_waited = g + 1
    assert groups_waited < groups

    @pl.loop(0, steps1)
    def _(i):
        for s in range(_SWEEPS):
            sweep = first_sweep + i * _SWEEPS + s
            read((sweep - _LAG, sweep))
        g = lax.div(i * _PAIRS1 + (_PAIRS1 - 1), group_pairs)

        @pl.when(i * _PAIRS1 <= g * group_pairs)
        def _():
            wait(group_rows, group_sems.at[g])

        compute(i * _PAIRS1, _PAIRS1)

    last_sweep = first_sweep + steps1 * _SWEEPS
    if last_sweep < sweeps - _LATE:
        pl.loop(last_sweep, sweeps - _LATE)(lambda i: read((i - _LAG, i)))
    for i in range(sweeps - _LATE, sweeps):
        read((i - _LAG, i), (None, late_sem))
    for i in range(sweeps - _LAG, sweeps):
        read((i, None), (late_sem if i >= sweeps - _LATE else None, None))

    late_rows = _LATE * group * _READ_PIECE
    for g in range(groups_waited, groups - 1):
        wait(group_rows, group_sems.at[g])
    wait(group_rows - late_rows, group_sems.at[groups - 1])
    for i in range(8):
        write(i)
    pl.loop(8, _LEAD)(write)
    wait(late_rows, late_sem)

    write_pairs = _WRITE_STREAMS * _STREAM // _PAIR
    for i in range(steps2):
        computed = steps1 * _PAIRS1 + i * _PAIRS2
        assert _LEAD + i * _WRITES <= computed // write_pairs * group_writes

    @pl.loop(0, steps2)
    def _(i):
        compute(steps1 * _PAIRS1 + i * _PAIRS2, _PAIRS2)

        @pl.when(i < steps2 - 1)
        def _():
            for s in range(_WRITES):
                write(_LEAD + i * _WRITES + s)

    pl.loop(_LEAD + (steps2 - 1) * _WRITES, writes)(write)
    wait(buf.shape[0], out_sem)


@jax.jit
def pallas_standalone__standard_2d_1d_3d_conv__vision_kernel(
    x: jax.Array,
    w: jax.Array,
    b: jax.Array,
):
    batch, height, width, cin = x.shape
    kh, kw, _, cout = w.shape
    assert (kh, kw) == (1, 1) and cin == cout == 3 * _LANES
    assert x.dtype == w.dtype == jnp.bfloat16
    rows = x.size // _LANES
    n_streams = rows // _STREAM
    groups = n_streams // sum(n for n, _ in _READ_COPIES)
    assert groups * sum(n for n, _ in _READ_COPIES) * _STREAM == rows
    assert n_streams % _WRITE_STREAMS == 0

    tiles = x.reshape(-1, 8, 3, _LANES).transpose(0, 2, 1, 3)
    hbm = pl.BlockSpec(memory_space=pltpu.HBM)
    out = pl.pallas_call(
        _conv1x1_kernel,
        in_specs=[hbm, hbm, hbm],
        out_specs=hbm,
        out_shape=jax.ShapeDtypeStruct((n_streams, _STREAM, _LANES), x.dtype),
        scratch_shapes=[
            pltpu.VMEM((rows, _LANES), x.dtype),
            pltpu.VMEM((cin, cout), w.dtype),
            pltpu.VMEM((cout,), b.dtype),
            pltpu.SemaphoreType.DMA((groups,)),
            pltpu.SemaphoreType.DMA(()),
            pltpu.SemaphoreType.DMA(()),
        ],
        compiler_params=pltpu.CompilerParams(
            vmem_limit_bytes=120 * 2**20,
            disable_bounds_checks=True,
            disable_semaphore_checks=True,
        ),
    )(tiles.reshape(n_streams, _STREAM, _LANES), w.reshape(cin, cout), b)
    out = out.reshape(-1, 3, 8, _LANES).transpose(0, 2, 1, 3)
    return out.reshape(batch, height, width, cout)
```

```python
import jax
import jax.numpy as jnp
from jax import lax
import jax.experimental.pallas as pl
import jax.experimental.pallas.tpu as pltpu

_LANES = 128
_STREAM = 4096
_PAIR = 48

_READ_PIECE = 32
_READ_COPIES = ((5, 1), (1, 0)) * 2
_LAG = 12
_SWEEPS = 12
_PAIRS1 = 48
_LATE = 5

_WRITE_PIECE = 64
_WRITE_STREAMS = 6
_LEAD = 16
_WRITES = 19
_PAIRS2 = 96

_DOT_PAIRS = 12


def _matmul(view, w_ref, bias):
    m = view.shape[0] // _PAIR
    regs = pltpu.bitcast(view[...], jnp.uint32).reshape(m, 3, 8, _LANES)
    low = lax.broadcasted_iota(jnp.int32, (m, 8, _LANES), 1) < 4

    def dot(first, second, k):
        lhs = jnp.where(low, regs[:, first], regs[:, second]).reshape(8 * m, _LANES)
        acc = jnp.dot(
            pltpu.bitcast(lhs, view.dtype),
            w_ref[pl.ds(k * _LANES, _LANES), :],
            preferred_element_type=jnp.float32,
        )
        return acc.reshape(m, 2, 8, 3 * _LANES)

    y0, y1, y2 = dot(0, 1, 0), dot(2, 0, 1), dot(1, 2, 2)
    a = y0[:, 0] + y1[:, 1] + y2[:, 0] + bias
    b = y0[:, 1] + y1[:, 0] + y2[:, 1] + bias
    tiles = [t[:, :, n * _LANES:(n + 1) * _LANES] for t in (a, b) for n in range(3)]
    out = jnp.stack(tiles, axis=1).reshape(view.shape)
    view[...] = out.astype(view.dtype)


def _conv1x1_kernel(
    x_hbm, w_hbm, b_hbm, o_hbm, buf, w_ref, b_ref, group_sems, late_sem, out_sem
):
    n_streams = x_hbm.shape[0]
    streams = buf.reshape(x_hbm.shape)
    pairs = buf.shape[0] // _PAIR

    group = sum(n for n, _ in _READ_COPIES)
    groups = n_streams // group
    group_rows = group * _STREAM
    group_sweeps = _STREAM // _READ_PIECE
    sweeps = groups * group_sweeps
    head = _LAG + (sweeps - _LATE - _LAG) % _SWEEPS
    idle_steps = pl.cdiv(group_sweeps + _LAG - head, _SWEEPS) + 2
    first_sweep = head + idle_steps * _SWEEPS
    steps1 = (sweeps - _LATE - first_sweep) // _SWEEPS
    steps1 -= (pairs - steps1 * _PAIRS1) % _PAIRS2 // _PAIRS1
    steps2 = (pairs - steps1 * _PAIRS1) // _PAIRS2
    assert steps1 * _PAIRS1 + steps2 * _PAIRS2 == pairs

    group_writes = _STREAM // _WRITE_PIECE
    writes = n_streams // _WRITE_STREAMS * group_writes

    def wait(rows, sem):
        size = buf.at[pl.ds(0, rows)]
        pltpu.make_async_copy(size, size, sem).wait()

    def locate(i, per_group, piece):
        if isinstance(i, int):
            return i // per_group, i % per_group * piece
        shift = per_group.bit_length() - 1
        return i >> shift, pl.multiple_of((i & (per_group - 1)) * piece, piece)

    def read(sweep_of_thread, sem_of_thread=(None, None)):
        first = 0
        for n, thread in _READ_COPIES:
            if sweep_of_thread[thread] is not None:
                g, row = locate(sweep_of_thread[thread], group_sweeps, _READ_PIECE)
                idx = (pl.ds(g * group + first, n), pl.ds(row, _READ_PIECE))
                sem = sem_of_thread[thread]
                if sem is None:
                    sem = group_sems.at[g]
                copy = pltpu.make_async_copy(x_hbm.at[idx], streams.at[idx], sem)
                copy.start(priority=thread)
            first += n

    def write(i):
        g, row = locate(i, group_writes, _WRITE_PIECE)
        idx = (pl.ds(g * _WRITE_STREAMS, _WRITE_STREAMS), pl.ds(row, _WRITE_PIECE))
        copy = pltpu.make_async_copy(streams.at[idx], o_hbm.at[idx], out_sem)
        copy.start(priority=1)

    def compute(first_pair, n_pairs):
        row = pl.multiple_of(first_pair * _PAIR, 16)
        view = buf.at[pl.ds(row, n_pairs * _PAIR)]
        for i in range(0, n_pairs, _DOT_PAIRS):
            _matmul(view.at[pl.ds(i * _PAIR, _DOT_PAIRS * _PAIR)], w_ref, bias)

    w_copy = pltpu.make_async_copy(w_hbm, w_ref, out_sem)
    b_copy = pltpu.make_async_copy(b_hbm, b_ref, out_sem)
    read((None, 0))
    pl.loop(1, _LAG)(lambda i: read((None, i)))
    w_copy.start()
    b_copy.start()
    pl.loop(_LAG, first_sweep)(lambda i: read((i - _LAG, i)))
    w_copy.wait()
    b_copy.wait()
    bias = b_ref[...].astype(jnp.float32).reshape(1, -1)

    group_pairs = group_rows // _PAIR
    for i in range(steps1):
        g = ((i + 1) * _PAIRS1 - 1) // group_pairs
        assert (g + 1) * group_sweeps + _LAG <= first_sweep + (i + 1) * _SWEEPS
    groups_waited = g + 1
    assert groups_waited < groups

    @pl.loop(0, steps1)
    def _(i):
        g = lax.div(i * _PAIRS1 + (_PAIRS1 - 1), group_pairs)

        @pl.when(i * _PAIRS1 <= g * group_pairs)
        def _():
            wait(group_rows, group_sems.at[g])

        for s in range(_SWEEPS):
            sweep = first_sweep + i * _SWEEPS + s
            read((sweep - _LAG, sweep))
        compute(i * _PAIRS1, _PAIRS1)

    last_sweep = first_sweep + steps1 * _SWEEPS
    if last_sweep < sweeps - _LATE:
        pl.loop(last_sweep, sweeps - _LATE)(lambda i: read((i - _LAG, i)))
    for i in range(sweeps - _LATE, sweeps):
        read((i - _LAG, i), (None, late_sem))
    for i in range(sweeps - _LAG, sweeps):
        read((i, None), (late_sem if i >= sweeps - _LATE else None, None))

    late_rows = _LATE * group * _READ_PIECE
    for g in range(groups_waited, groups - 1):
        wait(group_rows, group_sems.at[g])
    wait(group_rows - late_rows, group_sems.at[groups - 1])
    for i in range(8):
        write(i)
    pl.loop(8, _LEAD)(write)
    wait(late_rows, late_sem)

    write_pairs = _WRITE_STREAMS * _STREAM // _PAIR
    for i in range(steps2):
        computed = steps1 * _PAIRS1 + i * _PAIRS2
        assert _LEAD + (i + 1) * _WRITES <= computed // write_pairs * group_writes

    @pl.loop(0, steps2)
    def _(i):
        for s in range(_WRITES):
            write(_LEAD + i * _WRITES + s)
        compute(steps1 * _PAIRS1 + i * _PAIRS2, _PAIRS2)

    pl.loop(_LEAD + steps2 * _WRITES, writes)(write)
    wait(buf.shape[0], out_sem)


@jax.jit
def pallas_standalone__standard_2d_1d_3d_conv__vision_kernel(
    x: jax.Array,
    w: jax.Array,
    b: jax.Array,
):
    batch, height, width, cin = x.shape
    kh, kw, _, cout = w.shape
    assert (kh, kw) == (1, 1) and cin == cout == 3 * _LANES
    assert x.dtype == w.dtype == jnp.bfloat16
    rows = x.size // _LANES
    n_streams = rows // _STREAM
    groups = n_streams // sum(n for n, _ in _READ_COPIES)
    assert groups * sum(n for n, _ in _READ_COPIES) * _STREAM == rows
    assert n_streams % _WRITE_STREAMS == 0

    tiles = x.reshape(-1, 8, 3, _LANES).transpose(0, 2, 1, 3)
    hbm = pl.BlockSpec(memory_space=pltpu.HBM)
    out = pl.pallas_call(
        _conv1x1_kernel,
        in_specs=[hbm, hbm, hbm],
        out_specs=hbm,
        out_shape=jax.ShapeDtypeStruct((n_streams, _STREAM, _LANES), x.dtype),
        scratch_shapes=[
            pltpu.VMEM((rows, _LANES), x.dtype),
            pltpu.VMEM((cin, cout), w.dtype),
            pltpu.VMEM((cout,), b.dtype),
            pltpu.SemaphoreType.DMA((groups,)),
            pltpu.SemaphoreType.DMA(()),
            pltpu.SemaphoreType.DMA(()),
        ],
        compiler_params=pltpu.CompilerParams(
            vmem_limit_bytes=120 * 2**20,
            disable_bounds_checks=True,
            disable_semaphore_checks=True,
        ),
    )(tiles.reshape(n_streams, _STREAM, _LANES), w.reshape(cin, cout), b)
    out = out.reshape(-1, 3, 8, _LANES).transpose(0, 2, 1, 3)
    return out.reshape(batch, height, width, cout)
```

```python
import jax
import jax.numpy as jnp
from jax import lax
import jax.experimental.pallas as pl
import jax.experimental.pallas.tpu as pltpu

_LANES = 128
_PAIR = 48
_DOT_PAIRS = 12

_READ_STREAM = 2048
_READ_PIECE = 32
_READ_COPIES = ((3, 1), (3, 1), (2, 0)) * 3
_LAG = 13
_LATE = (9, 18)
_SWEEPS = 6
_PAIRS1 = 48

_WRITE_STREAM = 4096
_WRITE_PIECE = 64
_WRITE_GROUP = 6
_LEAD = 24
_WRITES = 19
_PAIRS2 = 96


def _matmul(view, w_ref, bias):
    m = view.shape[0] // _PAIR
    regs = pltpu.bitcast(view[...], jnp.uint32).reshape(m, 3, 8, _LANES)
    low = lax.broadcasted_iota(jnp.int32, (m, 8, _LANES), 1) < 4

    def dot(first, second, k):
        lhs = jnp.where(low, regs[:, first], regs[:, second]).reshape(8 * m, _LANES)
        acc = jnp.dot(
            pltpu.bitcast(lhs, view.dtype),
            w_ref[pl.ds(k * _LANES, _LANES), :],
            preferred_element_type=jnp.float32,
        )
        return acc.reshape(m, 2, 8, 3 * _LANES)

    y0, y1, y2 = dot(0, 1, 0), dot(2, 0, 1), dot(1, 2, 2)
    a = y0[:, 0] + y1[:, 1] + y2[:, 0] + bias
    b = y0[:, 1] + y1[:, 0] + y2[:, 1] + bias
    tiles = [t[:, :, n * _LANES:(n + 1) * _LANES] for t in (a, b) for n in range(3)]
    out = jnp.stack(tiles, axis=1).reshape(view.shape)
    view[...] = out.astype(view.dtype)


def _locate(i, group_sweeps, piece):
    if isinstance(i, int):
        return i // group_sweeps, i % group_sweeps * piece
    shift = group_sweeps.bit_length() - 1
    assert group_sweeps == 1 << shift
    return i >> shift, pl.multiple_of((i & (group_sweeps - 1)) * piece, piece)


def _conv1x1_kernel(
    x_hbm, w_hbm, b_hbm, o_hbm, buf, w_ref, b_ref, group_sems, late_sem, out_sem
):
    read_view = buf.reshape(x_hbm.shape)
    write_view = buf.reshape(o_hbm.shape)
    pairs = buf.shape[0] // _PAIR

    copies = ([], [])
    order = []
    group = 0
    for n, thread in _READ_COPIES:
        order.append((thread, len(copies[thread])))
        copies[thread].append((group, n))
        group += n
    groups = x_hbm.shape[0] // group
    group_rows = group * _READ_STREAM
    group_pairs = group_rows // _PAIR
    group_sweeps = _READ_STREAM // _READ_PIECE
    sweeps = groups * group_sweeps
    lag_sweeps = pl.cdiv(_LAG, len(copies[0]))
    tail = sweeps - pl.cdiv(_LATE[1], len(copies[1]))
    assert _LATE[0] <= _LAG

    steps1 = (tail - group_sweeps - lag_sweeps) // _SWEEPS - 2
    steps1 -= (pairs - steps1 * _PAIRS1) % _PAIRS2 // _PAIRS1
    steps2 = (pairs - steps1 * _PAIRS1) // _PAIRS2
    assert steps1 * _PAIRS1 + steps2 * _PAIRS2 == pairs
    first_sweep = tail - steps1 * _SWEEPS

    group_writes = _WRITE_STREAM // _WRITE_PIECE
    writes = o_hbm.shape[0] // _WRITE_GROUP * group_writes

    def wait(rows, sem):
        size = buf.at[pl.ds(0, rows)]
        pltpu.make_async_copy(size, size, sem).wait()

    late_rows = []

    def read(thread, sweep, copy):
        first, n = copies[thread][copy]
        g, row = _locate(sweep, group_sweeps, _READ_PIECE)
        sem = group_sems.at[g]
        if isinstance(sweep, int):
            if (sweeps - sweep) * len(copies[thread]) - copy <= _LATE[thread]:
                sem = late_sem
                late_rows.append(n * _READ_PIECE)
        idx = (pl.ds(g * group + first, n), pl.ds(row, _READ_PIECE))
        copy = pltpu.make_async_copy(x_hbm.at[idx], read_view.at[idx], sem)
        copy.start(priority=thread)

    def read_sweep(i):
        for thread, copy in order:
            shift = 0
            if thread == 0:
                shift, copy = divmod(copy - _LAG, len(copies[0]))
            if not isinstance(i, int) or 0 <= i + shift < sweeps:
                read(thread, i + shift, copy)

    def write(i):
        g, row = _locate(i, group_writes, _WRITE_PIECE)
        idx = (pl.ds(g * _WRITE_GROUP, _WRITE_GROUP), pl.ds(row, _WRITE_PIECE))
        copy = pltpu.make_async_copy(write_view.at[idx], o_hbm.at[idx], out_sem)
        copy.start(priority=1)

    def compute(first_pair, n_pairs):
        row = pl.multiple_of(first_pair * _PAIR, 16)
        view = buf.at[pl.ds(row, n_pairs * _PAIR)]
        for i in range(0, n_pairs, _DOT_PAIRS):
            _matmul(view.at[pl.ds(i * _PAIR, _DOT_PAIRS * _PAIR)], w_ref, bias)

    w_copy = pltpu.make_async_copy(w_hbm, w_ref, out_sem)
    b_copy = pltpu.make_async_copy(b_hbm, b_ref, out_sem)
    for i in range(lag_sweeps - 1):
        read_sweep(i)
    w_copy.start()
    b_copy.start()
    read_sweep(lag_sweeps - 1)
    pl.loop(lag_sweeps, first_sweep)(read_sweep)
    w_copy.wait()
    b_copy.wait()
    bias = b_ref[...].astype(jnp.float32).reshape(1, -1)

    for i in range(steps1):
        g = ((i + 1) * _PAIRS1 - 1) // group_pairs
        assert (g + 1) * group_sweeps + lag_sweeps <= first_sweep + i * _SWEEPS
    groups_waited = g + 1
    assert groups_waited < groups

    @pl.loop(0, steps1)
    def _(i):
        g = lax.div(i * _PAIRS1 + (_PAIRS1 - 1), group_pairs)

        @pl.when(i * _PAIRS1 <= g * group_pairs)
        def _():
            wait(group_rows, group_sems.at[g])

        for s in range(_SWEEPS):
            read_sweep(first_sweep + i * _SWEEPS + s)
        compute(i * _PAIRS1, _PAIRS1)

    for i in range(tail, sweeps + lag_sweeps):
        read_sweep(i)

    for g in range(groups_waited, groups - 1):
        wait(group_rows, group_sems.at[g])
    wait(group_rows - sum(late_rows), group_sems.at[groups - 1])
    for i in range(_LEAD):
        write(i)
    wait(sum(late_rows), late_sem)

    write_pairs = _WRITE_GROUP * _WRITE_STREAM // _PAIR
    for i in range(steps2):
        computed = steps1 * _PAIRS1 + i * _PAIRS2
        assert _LEAD + (i + 1) * _WRITES <= computed // write_pairs * group_writes

    @pl.loop(0, steps2)
    def _(i):
        for s in range(_WRITES):
            write(_LEAD + i * _WRITES + s)
        compute(steps1 * _PAIRS1 + i * _PAIRS2, _PAIRS2)

    pl.loop(_LEAD + steps2 * _WRITES, writes)(write)
    wait(buf.shape[0], out_sem)


@jax.jit
def pallas_standalone__standard_2d_1d_3d_conv__vision_kernel(
    x: jax.Array,
    w: jax.Array,
    b: jax.Array,
):
    batch, height, width, cin = x.shape
    kh, kw, _, cout = w.shape
    assert (kh, kw) == (1, 1) and cin == cout == 3 * _LANES
    assert x.dtype == w.dtype == jnp.bfloat16
    rows = x.size // _LANES
    group_rows = sum(n for n, _ in _READ_COPIES) * _READ_STREAM
    assert rows % group_rows == 0 and rows % (_WRITE_GROUP * _WRITE_STREAM) == 0

    tiles = x.reshape(-1, 8, 3, _LANES).transpose(0, 2, 1, 3)
    hbm = pl.BlockSpec(memory_space=pltpu.HBM)
    out = pl.pallas_call(
        _conv1x1_kernel,
        in_specs=[hbm, hbm, hbm],
        out_specs=hbm,
        out_shape=jax.ShapeDtypeStruct(
            (rows // _WRITE_STREAM, _WRITE_STREAM, _LANES), x.dtype
        ),
        scratch_shapes=[
            pltpu.VMEM((rows, _LANES), x.dtype),
            pltpu.VMEM((cin, cout), w.dtype),
            pltpu.VMEM((cout,), b.dtype),
            pltpu.SemaphoreType.DMA((rows // group_rows,)),
            pltpu.SemaphoreType.DMA(()),
            pltpu.SemaphoreType.DMA(()),
        ],
        compiler_params=pltpu.CompilerParams(
            vmem_limit_bytes=120 * 2**20,
            disable_bounds_checks=True,
            disable_semaphore_checks=True,
        ),
    )(tiles.reshape(-1, _READ_STREAM, _LANES), w.reshape(cin, cout), b)
    out = out.reshape(-1, 3, 8, _LANES).transpose(0, 2, 1, 3)
    return out.reshape(batch, height, width, cout)
```

```python
import jax
import jax.numpy as jnp
from jax import lax
import jax.experimental.pallas as pl
import jax.experimental.pallas.tpu as pltpu

_LANES = 128
_PAIR = 48
_DOT_PAIRS = 12

_READ_STREAM = 2048
_READ_PIECE = 32
_READ_COPIES = ((3, 1), (3, 1), (2, 0)) * 3
_LAG = 13
_LATE = (9, 18)
_SWEEPS = 6
_SETTLE = 16
_PAIRS1 = 48

_WRITE_STREAM = 4096
_WRITE_PIECE = 64
_WRITE_GROUP = 6
_LEAD = 24
_WRITES = 19
_PAIRS2 = 96


def _matmul(view, w_ref, bias):
    m = view.shape[0] // _PAIR
    regs = pltpu.bitcast(view[...], jnp.uint32).reshape(m, 3, 8, _LANES)
    low = lax.broadcasted_iota(jnp.int32, (m, 8, _LANES), 1) < 4

    def dot(first, second, k):
        lhs = jnp.where(low, regs[:, first], regs[:, second]).reshape(8 * m, _LANES)
        acc = jnp.dot(
            pltpu.bitcast(lhs, view.dtype),
            w_ref[pl.ds(k * _LANES, _LANES), :],
            preferred_element_type=jnp.float32,
        )
        return acc.reshape(m, 2, 8, 3 * _LANES)

    y0, y1, y2 = dot(0, 1, 0), dot(2, 0, 1), dot(1, 2, 2)
    a = y0[:, 0] + y1[:, 1] + y2[:, 0] + bias
    b = y0[:, 1] + y1[:, 0] + y2[:, 1] + bias
    tiles = [t[:, :, n * _LANES:(n + 1) * _LANES] for t in (a, b) for n in range(3)]
    out = jnp.stack(tiles, axis=1).reshape(view.shape)
    view[...] = out.astype(view.dtype)


def _locate(i, group_sweeps, piece):
    if isinstance(i, int):
        return i // group_sweeps, i % group_sweeps * piece
    shift = group_sweeps.bit_length() - 1
    assert group_sweeps == 1 << shift
    return i >> shift, pl.multiple_of((i & (group_sweeps - 1)) * piece, piece)


def _conv1x1_kernel(x_hbm, w_hbm, b_hbm, o_hbm, buf, w_ref, b_ref, sems):
    read_view = buf.reshape(x_hbm.shape)
    write_view = buf.reshape(o_hbm.shape)
    pairs = buf.shape[0] // _PAIR

    copies = ([], [])
    order = []
    group = 0
    for n, thread in _READ_COPIES:
        order.append((thread, len(copies[thread])))
        copies[thread].append((group, n))
        group += n
    groups = x_hbm.shape[0] // group
    group_rows = group * _READ_STREAM
    group_pairs = group_rows // _PAIR
    group_sweeps = _READ_STREAM // _READ_PIECE
    sweeps = groups * group_sweeps
    lag_sweeps = pl.cdiv(_LAG, len(copies[0]))
    tail = sweeps - pl.cdiv(_LATE[1], len(copies[1]))
    assert _LATE[0] <= _LAG

    steps1 = (tail - group_sweeps - _SETTLE) // _SWEEPS
    steps1 -= (pairs - steps1 * _PAIRS1) % _PAIRS2 // _PAIRS1
    steps2 = (pairs - steps1 * _PAIRS1) // _PAIRS2
    assert steps1 * _PAIRS1 + steps2 * _PAIRS2 == pairs
    first_sweep = tail - steps1 * _SWEEPS

    group_writes = _WRITE_STREAM // _WRITE_PIECE
    writes = o_hbm.shape[0] // _WRITE_GROUP * group_writes

    def wait(rows, sem):
        size = buf.at[pl.ds(0, rows)]
        pltpu.make_async_copy(size, size, sem).wait()

    last_sem, late_sem = sems.at[(groups - 1) % 2], sems.at[groups % 2]
    late_rows = []

    def read(thread, sweep, copy):
        first, n = copies[thread][copy]
        g, row = _locate(sweep, group_sweeps, _READ_PIECE)
        sem = sems.at[g & 1]
        if isinstance(sweep, int):
            if (sweeps - sweep) * len(copies[thread]) - copy <= _LATE[thread]:
                sem = late_sem
                late_rows.append(n * _READ_PIECE)
        idx = (pl.ds(g * group + first, n), pl.ds(row, _READ_PIECE))
        copy = pltpu.make_async_copy(x_hbm.at[idx], read_view.at[idx], sem)
        copy.start(priority=thread)

    def read_sweep(i):
        for thread, copy in order:
            shift = 0
            if thread == 0:
                shift, copy = divmod(copy - _LAG, len(copies[0]))
            if not isinstance(i, int) or 0 <= i + shift < sweeps:
                read(thread, i + shift, copy)

    def write(i):
        g, row = _locate(i, group_writes, _WRITE_PIECE)
        idx = (pl.ds(g * _WRITE_GROUP, _WRITE_GROUP), pl.ds(row, _WRITE_PIECE))
        copy = pltpu.make_async_copy(write_view.at[idx], o_hbm.at[idx], last_sem)
        copy.start(priority=1)

    def compute(first_pair, n_pairs):
        row = pl.multiple_of(first_pair * _PAIR, 16)
        view = buf.at[pl.ds(row, n_pairs * _PAIR)]
        for i in range(0, n_pairs, _DOT_PAIRS):
            _matmul(view.at[pl.ds(i * _PAIR, _DOT_PAIRS * _PAIR)], w_ref, bias)

    w_copy = pltpu.make_async_copy(w_hbm, w_ref, sems.at[1])
    b_copy = pltpu.make_async_copy(b_hbm, b_ref, sems.at[1])
    for i in range(lag_sweeps - 1):
        read_sweep(i)
    w_copy.start()
    b_copy.start()
    read_sweep(lag_sweeps - 1)
    pl.loop(lag_sweeps, group_sweeps)(read_sweep)
    w_copy.wait()
    b_copy.wait()
    pl.loop(group_sweeps, first_sweep)(read_sweep)
    bias = b_ref[...].astype(jnp.float32).reshape(1, -1)

    assert lag_sweeps <= _SETTLE <= group_sweeps - 2 * _SWEEPS
    assert first_sweep - _SETTLE - group_sweeps < _SWEEPS
    for i in range(steps1):
        landed = (first_sweep + i * _SWEEPS - _SETTLE) // group_sweeps
        assert (i + 1) * _PAIRS1 <= landed * group_pairs
    assert landed == groups - 1

    @pl.loop(0, steps1)
    def _(i):
        sweep = first_sweep + i * _SWEEPS
        g, row = _locate(sweep - _SETTLE, group_sweeps, _READ_PIECE)

        @pl.when(row < _SWEEPS * _READ_PIECE)
        def _():
            wait(group_rows, sems.at[(g - 1) & 1])

        for s in range(_SWEEPS):
            read_sweep(sweep + s)
        compute(i * _PAIRS1, _PAIRS1)

    for i in range(tail, sweeps + lag_sweeps):
        read_sweep(i)

    wait(group_rows - sum(late_rows), last_sem)
    for i in range(_LEAD):
        write(i)
    wait(sum(late_rows), late_sem)

    write_pairs = _WRITE_GROUP * _WRITE_STREAM // _PAIR
    for i in range(steps2):
        computed = steps1 * _PAIRS1 + i * _PAIRS2
        assert _LEAD + (i + 1) * _WRITES <= computed // write_pairs * group_writes

    @pl.loop(0, steps2)
    def _(i):
        for s in range(_WRITES):
            write(_LEAD + i * _WRITES + s)
        compute(steps1 * _PAIRS1 + i * _PAIRS2, _PAIRS2)

    pl.loop(_LEAD + steps2 * _WRITES, writes)(write)
    wait(buf.shape[0], last_sem)


@jax.jit
def pallas_standalone__standard_2d_1d_3d_conv__vision_kernel(
    x: jax.Array,
    w: jax.Array,
    b: jax.Array,
):
    batch, height, width, cin = x.shape
    kh, kw, _, cout = w.shape
    assert (kh, kw) == (1, 1) and cin == cout == 3 * _LANES
    assert x.dtype == w.dtype == jnp.bfloat16
    rows = x.size // _LANES
    group_rows = sum(n for n, _ in _READ_COPIES) * _READ_STREAM
    assert rows % group_rows == 0 and rows % (_WRITE_GROUP * _WRITE_STREAM) == 0

    tiles = x.reshape(-1, 8, 3, _LANES).transpose(0, 2, 1, 3)
    hbm = pl.BlockSpec(memory_space=pltpu.HBM)
    out = pl.pallas_call(
        _conv1x1_kernel,
        in_specs=[hbm, hbm, hbm],
        out_specs=hbm,
        out_shape=jax.ShapeDtypeStruct(
            (rows // _WRITE_STREAM, _WRITE_STREAM, _LANES), x.dtype
        ),
        scratch_shapes=[
            pltpu.VMEM((rows, _LANES), x.dtype),
            pltpu.VMEM((cin, cout), w.dtype),
            pltpu.VMEM((cout,), b.dtype),
            pltpu.SemaphoreType.DMA((2,)),
        ],
        compiler_params=pltpu.CompilerParams(
            vmem_limit_bytes=120 * 2**20,
            disable_bounds_checks=True,
        ),
    )(tiles.reshape(-1, _READ_STREAM, _LANES), w.reshape(cin, cout), b)
    out = out.reshape(-1, 3, 8, _LANES).transpose(0, 2, 1, 3)
    return out.reshape(batch, height, width, cout)
```
